```python
import jax
import jax.numpy as jnp

def _softmax(x, axis=-1):
    return jax.nn.softmax(x, axis=axis)

def _gelu(x):
    return jax.nn.gelu(x, approximate=True)

def _silu(x):
    return jax.nn.silu(x)

def _sigmoid(x):
    return jax.nn.sigmoid(x)

def _layernorm(x, axis=-1, eps=1e-05):
    m = jnp.mean(x, axis=axis, keepdims=True)
    v = jnp.var(x, axis=axis, keepdims=True)
    return (x - m) / jnp.sqrt(v + eps)

def _scatter_add(tgt, idx, src, axis=0):
    return tgt.at[idx].add(src)

def _segment_sum(src, seg, n):
    return jax.ops.segment_sum(src, seg, n)

class _Rng:

    def __init__(self, key):
        self._k = key

    def _next(self):
        self._k, sub = jax.random.split(self._k)
        return sub

    def normal(self, shape):
        return jax.random.normal(self._next(), shape, dtype=jnp.bfloat16)

    def randint(self, lo, hi, shape):
        return jax.random.randint(self._next(), shape, lo, hi, dtype=jnp.int32)

    def uniform(self, shape, lo=0.0, hi=1.0):
        return jax.random.uniform(self._next(), shape, jnp.bfloat16, lo, hi)

    def permutation(self, n):
        return jax.random.permutation(self._next(), n)
kernel_name = 'standalone__window_attn_davit__vision'

def setup_inputs():
    _rng = _Rng(jax.random.key(int.from_bytes(__import__("os").urandom(4), "little")))
    _w = lambda a: (lambda t: t.astype(jnp.bfloat16) if jnp.issubdtype(t.dtype, jnp.floating) else t)(jnp.asarray(a))
    HW = 512
    C0 = 192
    ws = 7
    nh = 4
    H = W = max(HW // ws * ws, ws)
    C = max(C0 // nh * nh, nh)
    k = 3
    return {'x': _w((lambda *s: _rng.normal(s) * 0.05)(1, H, W, C)), 'dw_pe': _w((lambda *s: _rng.normal(s) * 0.05)(k, k, C) * 0.1), 'w_qkv': _w((lambda *s: _rng.normal(s) * 0.05)(C, 3 * C) * C ** (-0.5)), 'w_o': _w((lambda *s: _rng.normal(s) * 0.05)(C, C) * C ** (-0.5))}

def reference(x, dw_pe, w_qkv, w_o):
    B, H, W, C = x.shape
    ws = 7
    nh = 4
    dh = C // nh
    kk = dw_pe.shape[0]
    pad = kk // 2
    xp = jnp.pad(x, ((0, 0), (pad, pad), (pad, pad), (0, 0)))
    pe = jnp.zeros_like(x)
    for i in range(kk):
        for j in range(kk):
            pe = pe + xp[:, i:i + H, j:j + W, :] * dw_pe[i, j][None, None, None, :]
    x0 = x + pe
    h = _layernorm(x0, axis=-1)
    hw = h.reshape(B, H // ws, ws, W // ws, ws, C)
    hw = (lambda x, *d: x.transpose(*d))(hw, 0, 1, 3, 2, 4, 5)
    hw = hw.reshape(-1, ws * ws, C)
    qkv = (hw @ w_qkv).reshape(-1, ws * ws, 3, nh, dh)
    q = qkv[:, :, 0].copy()
    k = qkv[:, :, 1].copy()
    v = qkv[:, :, 2].copy()
    scale = dh ** (-0.5)
    attn = jnp.einsum('wnhd,wmhd->whnm', q, k) * scale
    attn = _softmax(attn, axis=-1)
    out = jnp.einsum('whnm,wmhd->wnhd', attn, v)
    out = out.reshape(-1, ws * ws, C) @ w_o
    out = out.reshape(B, H // ws, W // ws, ws, ws, C)
    out = (lambda x, *d: x.transpose(*d))(out, 0, 1, 3, 2, 4, 5)
    out = out.reshape(B, H, W, C)
    return x0 + out
```

```python
import numpy as np
import jax
import jax.numpy as jnp
from jax import lax
import jax.experimental.pallas as pl
import jax.experimental.pallas.tpu as pltpu

WS = 7
NH = 4
C = 192
DH = C // NH
WL = 512
NT = 5
RP = 528
NPAIR = 37
LOG2E = 1.4426950408889634
GS = 2
LAG = 5


def _qkv_layout():
    src = -np.ones((NT * 128,), np.int64)
    q = lambda h: h * DH + np.arange(DH)
    k = lambda h: C + h * DH + np.arange(DH)
    v = lambda h: 2 * C + h * DH + np.arange(DH)
    src[0:48] = q(0); src[48:96] = q(1); src[96:128] = v(2)[:32]
    src[128:160] = v(3)[:32]; src[160:208] = q(2); src[208:256] = q(3)
    src[256:304] = k(0); src[304:352] = k(1)
    src[416:464] = k(2); src[464:512] = k(3)
    src[512:512 + 48] = v(0); src[512 + 48:512 + 64] = v(2)[32:]
    src[512 + 64:512 + 80] = v(3)[32:]; src[512 + 80:512 + 128] = v(1)
    return src


def _att_layout():
    src = -np.ones((256,), np.int64)
    ch = lambda h: h * DH + np.arange(DH)
    src[0:48] = ch(0); src[80:128] = ch(1)
    src[128:160] = ch(3)[:32]; src[128 + 48:128 + 64] = ch(2)[32:]; src[128 + 64:128 + 80] = ch(3)[32:]
    src[128 + 96:256] = ch(2)[:32]
    return src


def _consts():
    import ml_dtypes
    s = _qkv_layout()
    pm = np.zeros((3 * C, NT * 128), np.float32)
    cols = np.nonzero(s >= 0)[0]
    pm[s[cols], cols] = 1.0
    a = _att_layout()
    pa = np.zeros((C, 256), np.float32)
    cols = np.nonzero(a >= 0)[0]
    pa[a[cols], cols] = 1.0
    return pm.astype(ml_dtypes.bfloat16), pa.astype(ml_dtypes.bfloat16)


def _kernel(xa_ref, xm_ref, xb_ref, dw_ref, wqkv_ref, wo_ref, pm_ref, pa_ref, o_ref,
            dwb_scr, wq_scr, wo_scr, x0_scr, qkv_scr, att_scr):
    step = pl.program_id(0)
    nstrip = pl.num_programs(0) - 1
    s = step
    f32, bf16 = jnp.float32, jnp.bfloat16
    NTL = WL // 128

    @pl.when(step == 0)
    def _init():
        wp = jnp.dot(wqkv_ref[...], pm_ref[...], preferred_element_type=f32)
        col = lax.broadcasted_iota(jnp.int32, (C, NT * 128), 1)
        isq = (col < 96) | ((col >= 160) & (col < 256))
        wp = jnp.where(isq, wp * (DH ** -0.5 * LOG2E), wp)
        wq_scr[...] = wp.astype(bf16)
        wot = lax.dot_general(wo_ref[...], pa_ref[...], (((0,), (0,)), ((), ())),
                              preferred_element_type=f32)
        wo_scr[...] = wot.astype(bf16)
        dw = dw_ref[...].astype(f32)
        for k in range(9):
            wk = dw[:, k:k + 1]
            if k == 4:
                wk = wk + 1.0
            dwb_scr[k] = jnp.broadcast_to(wk, (C, 128))
        qkv_scr[:, :, pl.ds(WL, RP - WL), :] = jnp.zeros((WS, NT + 1, RP - WL, 128), f32)
        att_scr[...] = jnp.zeros(att_scr.shape, f32)
        x0_scr[...] = jnp.zeros(x0_scr.shape, f32)

    lane8 = lax.broadcasted_iota(jnp.int32, (8, 128), 1)
    lastm = lane8 < 127
    first = lane8 == 0

    def load_x(row, g, t):
        rows = pl.ds((g // 2) * 16, 16)
        ls = pl.ds(t * 128, 128)
        if row < 0:
            v, valid = xa_ref[0, rows, ls], s > 0
        elif row >= WS:
            v, valid = xb_ref[0, rows, ls], s < nstrip - 1
        else:
            v, valid = xm_ref[row, rows, ls], None
        v = v.astype(f32)[(g % 2) * 8:(g % 2) * 8 + 8]
        if t == NTL - 1:
            valid = lastm if valid is None else (lastm & valid)
        if valid is not None:
            v = jnp.where(valid, v, 0.0)
        return v

    def conv(r):
        acc = [None] * NTL
        for g in range(C // 8):
            rows = pl.ds(g * 8, 8)
            w = [dwb_scr[k, rows, :] for k in range(9)]
            part = r0p = r2p = None
            for t in range(NTL + 1):
                if t < NTL:
                    xa, xb, xc = [load_x(q, g, t) for q in (r - 1, r, r + 1)]
                    t0 = xa * w[0] + xb * w[3] + xc * w[6]
                    t1 = xa * w[1] + xb * w[4] + xc * w[7]
                    t2 = xa * w[2] + xb * w[5] + xc * w[8]
                    r0 = pltpu.roll(t0, 1, 1)
                    r2 = pltpu.roll(t2, 127, 1)
                if t > 0:
                    if t < NTL:
                        x0 = part + jnp.where(lastm, r2p, r2)
                    else:
                        x0 = part + r2p
                    x0_scr[r, rows, pl.ds((t - 1) * 128, 128)] = x0
                    acc[t - 1] = x0 if acc[t - 1] is None else acc[t - 1] + x0
                if t < NTL:
                    part = t1 + jnp.where(first, 0.0 if t == 0 else r0p, r0)
                    r0p, r2p = r0, r2
        return acc

    def ln(r, acc):
        tiles = []
        for t in range(NTL):
            ls = pl.ds(t * 128, 128)
            mean = jnp.sum(acc[t], axis=0, keepdims=True) * (1.0 / C)
            mean = jnp.broadcast_to(mean, (8, 128))
            acc2 = None
            for g in range(C // 8):
                d = x0_scr[r, pl.ds(g * 8, 8), ls] - mean
                acc2 = d * d if acc2 is None else acc2 + d * d
            var = jnp.sum(acc2, axis=0, keepdims=True) * (1.0 / C)
            rstd = jnp.broadcast_to(lax.rsqrt(var + 1e-5), (8, 128))
            hh = [(x0_scr[r, pl.ds(g * 8, 8), ls] - mean) * rstd for g in range(C // 8)]
            tiles.append(jnp.concatenate(hh, axis=0).astype(bf16))
        return tiles

    def proj(r, tiles):
        hT = jnp.concatenate(tiles, axis=1)
        qkv = lax.dot_general(hT, wq_scr[...], (((0,), (0,)), ((), ())), preferred_element_type=f32)
        tl = [qkv[:, n * 128:(n + 1) * 128] for n in range(NT)]
        for n in range(NT):
            qkv_scr[r, n, pl.ds(0, WL), :] = tl[n]
        lw = lax.broadcasted_iota(jnp.int32, (WL, 128), 1)
        qkv_scr[r, NT, pl.ds(0, WL), :] = jnp.where(lw >= 96, tl[0], jnp.where(lw < 32, tl[1], tl[4]))

    def stage_c(r):
        a = jnp.concatenate([att_scr[r, 0, pl.ds(0, WL), :], att_scr[r, 1, pl.ds(0, WL), :]], axis=1).astype(bf16)
        outT = lax.dot_general(wo_scr[...], a, (((1,), (1,)), ((), ())), preferred_element_type=f32)
        o_ref[r] = (x0_scr[r] + outT).astype(o_ref.dtype)

    lane = lax.broadcasted_iota(jnp.int32, (56, 128), 1)
    pad = lax.broadcasted_iota(jnp.int32, (8, 128), 0) == 7
    z8 = jnp.zeros((8, 128), f32)

    def softmax_t(st):
        v = [st[8 * a:8 * a + 8] for a in range(WS)]
        m = jnp.maximum(jnp.maximum(jnp.maximum(v[0], v[1]), jnp.maximum(v[2], v[3])),
                        jnp.maximum(jnp.maximum(v[4], v[5]), v[6]))
        m = jnp.max(jnp.where(pad, -jnp.inf, m), axis=0, keepdims=True)
        m = jnp.where(pad, jnp.inf, jnp.broadcast_to(m, (8, 128)))
        e = [jnp.exp2(v[a] - m) for a in range(WS)]
        l = ((e[0] + e[1]) + (e[2] + e[3])) + ((e[4] + e[5]) + e[6])
        l = jnp.sum(l, axis=0, keepdims=True)
        rl = jnp.broadcast_to(pl.reciprocal(l, approx=False, full_range=False), (8, 128))
        return jnp.concatenate([e[a] * rl for a in range(WS)], axis=0)

    def win(base, t, i):
        return jnp.concatenate([qkv_scr[r, t, pl.ds(base + WS * i, 8), :] for r in range(WS)], axis=0)

    def head_masks(p):
        off = 0 if p == 0 else 32
        return (lane >= off) & (lane < off + 48), (lane >= off + 48) & (lane < off + 96)

    def s_phase(base, p):
        ma, mb = head_masks(p)
        pts = []
        for i in range(2):
            m1, m2 = (ma, mb) if i == 0 else (mb, ma)
            q = win(base, p, i)
            qbd = jnp.concatenate([jnp.where(m1, q, 0.0), z8, jnp.where(m2, q, 0.0), z8], axis=0)
            kk = jnp.concatenate([win(base, 2 + p, i), z8], axis=0).astype(bf16)
            st = lax.dot_general(kk, qbd.astype(bf16), (((1,), (1,)), ((), ())),
                                 preferred_element_type=f32)[:56]
            pts += [softmax_t(st), z8]
        return jnp.concatenate(pts, axis=0).astype(bf16).T

    def pv_phase(base, p, U):
        T4 = [win(base, 4 + p, i) for i in range(2)]
        if p == 0:
            ma, _ = head_masks(0)
            va = [jnp.where(ma, T4[i], 0.0) for i in range(2)]
            vb = [jnp.where(lane >= 80, T4[i], 0.0) for i in range(2)]
            oa = ma
        else:
            la = (lane >= 48) & (lane < 64)
            lb = (lane >= 64) & (lane < 80)
            oa = (lane >= 96) | la
            ob = (lane < 32) | lb
            va = [jnp.where(oa, T4[i], 0.0) for i in range(2)]
            vb = [jnp.where(ob, T4[i], 0.0) for i in range(2)]
        v1 = jnp.concatenate([va[0], z8, vb[1], z8], axis=0).astype(bf16)
        v2 = jnp.concatenate([vb[0], z8, va[1], z8], axis=0).astype(bf16)
        o1 = jnp.dot(U[0:64], v1, preferred_element_type=f32)[:56]
        o2 = jnp.dot(U[64:128], v2, preferred_element_type=f32)[:56]
        a0 = jnp.where(oa, o1, o2)
        a1 = jnp.where(oa, o2, o1)
        for r in range(WS):
            att_scr[r, p, pl.ds(base, 8), :] = a0[8 * r:8 * r + 8]
            att_scr[r, p, pl.ds(base + WS, 8), :] = a1[8 * r:8 * r + 8]

    def stage_b():
        items = [(k * 2 * WS, p) for k in range(NPAIR) for p in (1, 0)]
        groups = [items[i:i + GS] for i in range(0, len(items), GS)]
        us = {}
        for g in range(len(groups) + LAG):
            if g < len(groups):
                for it in groups[g]:
                    us[it] = s_phase(*it)
            if g >= LAG:
                for it in groups[g - LAG]:
                    pv_phase(*it, us.pop(it))

    @pl.when(step < nstrip)
    def _main():
        stage_c(0)
        tiles = ln(0, conv(0))
        for r in range(1, WS):
            stage_c(r)
        for r in range(1, WS):
            acc = conv(r)
            proj(r - 1, tiles)
            tiles = ln(r, acc)
        proj(WS - 1, tiles)
        stage_b()

    @pl.when(step == nstrip)
    def _drain():
        for r in range(WS):
            stage_c(r)


@jax.jit
def pallas_standalone__window_attn_davit__vision_kernel(x, dw_pe, w_qkv, w_o):
    B, H, W, Cc = x.shape
    assert B == 1 and W == 511 and Cc == C and H % WS == 0 and dw_pe.shape == (3, 3, C)
    xt = jnp.transpose(x, (0, 1, 3, 2)).reshape(H, C, W)
    dwt = jnp.transpose(dw_pe.reshape(9, C))
    pm, pa = _consts()
    ns = H // WS
    grid_spec = pltpu.PrefetchScalarGridSpec(
        num_scalar_prefetch=0,
        grid=(ns + 1,),
        in_specs=[
            pl.BlockSpec((1, C, WL), lambda s: (jnp.maximum(jnp.minimum(s, ns - 1) * WS - 1, 0), 0, 0)),
            pl.BlockSpec((WS, C, WL), lambda s: (jnp.minimum(s, ns - 1), 0, 0)),
            pl.BlockSpec((1, C, WL), lambda s: (jnp.minimum(jnp.minimum(s, ns - 1) * WS + WS, H - 1), 0, 0)),
            pl.BlockSpec((C, 9), lambda s: (0, 0)),
            pl.BlockSpec((C, 3 * C), lambda s: (0, 0)),
            pl.BlockSpec((C, C), lambda s: (0, 0)),
            pl.BlockSpec((3 * C, NT * 128), lambda s: (0, 0)),
            pl.BlockSpec((C, 256), lambda s: (0, 0)),
        ],
        out_specs=pl.BlockSpec((WS, C, WL), lambda s: (jnp.maximum(s - 1, 0), 0, 0)),
        scratch_shapes=[
            pltpu.VMEM((9, C, 128), jnp.float32),
            pltpu.VMEM((C, NT * 128), jnp.bfloat16),
            pltpu.VMEM((C, 256), jnp.bfloat16),
            pltpu.VMEM((WS, C, WL), jnp.float32),
            pltpu.VMEM((WS, NT + 1, RP, 128), jnp.float32),
            pltpu.VMEM((WS, 2, RP, 128), jnp.float32),
        ],
    )
    out = pl.pallas_call(
        _kernel,
        grid_spec=grid_spec,
        out_shape=jax.ShapeDtypeStruct((H, C, W), x.dtype),
        compiler_params=pltpu.CompilerParams(
            dimension_semantics=("arbitrary",),
            vmem_limit_bytes=100 * 1024 * 1024,
        ),
    )(xt, xt, xt, dwt, w_qkv, w_o, pm, pa)
    return jnp.transpose(out.reshape(B, H, C, W), (0, 1, 3, 2))
```
